```python
import os as _os
_os.environ.setdefault("JAX_PLATFORMS", "cpu")
import jax
import jax.numpy as jnp

def _softmax(x, axis=-1):
    return jax.nn.softmax(x, axis=axis)
def _gelu(x):
    return jax.nn.gelu(x, approximate=True)
def _silu(x):
    return jax.nn.silu(x)
def _sigmoid(x):
    return jax.nn.sigmoid(x)
def _layernorm(x, axis=-1, eps=1e-5):
    m = jnp.mean(x, axis=axis, keepdims=True)
    v = jnp.var(x, axis=axis, keepdims=True)
    return (x - m) / jnp.sqrt(v + eps)
def _scatter_add(tgt, idx, src, axis=0):
    return tgt.at[idx].add(src)
def _segment_sum(src, seg, n):
    return jax.ops.segment_sum(src, seg, n)
class _Rng:
    def __init__(self, key):
        self._k = key
    def _next(self):
        self._k, sub = jax.random.split(self._k)
        return sub
    def normal(self, shape):
        return jax.random.normal(self._next(), shape, dtype=jnp.bfloat16)
    def randint(self, lo, hi, shape):
        return jax.random.randint(self._next(), shape, lo, hi, dtype=jnp.int32)
    def uniform(self, shape, lo=0.0, hi=1.0):
        return jax.random.uniform(self._next(), shape, jnp.bfloat16, lo, hi)
    def permutation(self, n):
        return jax.random.permutation(self._next(), n)


kernel_name = 'standalone__gqa_softmax__near_ridge'

def setup_inputs():
    _rng = _Rng(jax.random.key(int.from_bytes(__import__("os").urandom(4), "little")))
    _w = (lambda a: (lambda t: t.astype(jnp.bfloat16) if jnp.issubdtype(t.dtype, jnp.floating) else t)(jnp.asarray(a)))
    B, Hq, Hkv, Sq, Sk, D = 8, 16, 8, 160, 2048, 256
    return {
        "q": _w((lambda *s: _rng.normal(s) * 0.05)(B, Hq, Sq, D)),
        "k": _w((lambda *s: _rng.normal(s) * 3.2)(B, Hkv, Sk, D)),
        "v": _w((lambda *s: _rng.normal(s) * 0.05)(B, Hkv, Sk, D)),
    }

def reference(q, k, v):
    B, Hq, Sq, D = q.shape
    Hkv = k.shape[1]
    rep = Hq // Hkv
    k = jnp.repeat(k, rep, axis=1)
    v = jnp.repeat(v, rep, axis=1)
    scale = D ** -0.5
    scores = jnp.einsum("bhqd,bhkd->bhqk", q, k) * scale
    p = _softmax(scores, axis=-1)
    return jnp.einsum("bhqk,bhkd->bhqd", p, v)
```

```python
import functools
import math
import jax
import jax.numpy as jnp
import jax.experimental.pallas as pl
import jax.experimental.pallas.tpu as pltpu

KC = 256
NG = 4
NB = 6
LAST = 128
NT = (((1,), (1,)), ((), ()))


def _kernel(q_hbm, k_hbm, v_hbm, o_ref, qbuf, kbuf, vbuf, s_ref, m_ref, qsem, ksem, vsem,
            *, scale, NS):
    t = pl.program_id(0)
    _, M, Sk = s_ref.shape
    nk = Sk // KC
    slot = t % 2
    nslot = 1 - slot

    def q_copy(step, sl, u):
        return pltpu.make_async_copy(q_hbm.at[step * NG + u], qbuf.at[sl, u], qsem.at[sl, u])

    def k_copy(step, sl, u):
        return pltpu.make_async_copy(k_hbm.at[step * NG + u], kbuf.at[sl, u], ksem.at[sl, u])

    def v_copy(step, sl, u):
        return pltpu.make_async_copy(v_hbm.at[step * NG + u], vbuf.at[sl, u], vsem.at[sl, u])

    def pv(u):
        m = m_ref[u]
        mt = jnp.concatenate([m] * (KC // 128), axis=1)
        o = None
        l = None
        for j in range(nk):
            pf = jnp.exp2(s_ref[u, :, j * KC:(j + 1) * KC] - mt)
            for c in range(KC // 128):
                pc = pf[:, c * 128:(c + 1) * 128]
                l = pc if l is None else l + pc
            d = jnp.dot(pf.astype(jnp.bfloat16), vbuf[slot, u, j * KC:(j + 1) * KC, :],
                        preferred_element_type=jnp.float32)
            o = d if o is None else o + d
        l = jnp.sum(l, axis=-1, keepdims=True)
        o_ref[u] = (o / l).astype(o_ref.dtype)

    def qk(u, r0, r1):
        s = jax.lax.dot_general(qbuf[slot, u, r0:r1, :], kbuf[slot, u], NT,
                                preferred_element_type=jnp.float32) * scale
        s_ref[u, r0:r1, :] = s
        m_ref[u, r0:r1, :] = jnp.broadcast_to(jnp.max(s, axis=-1, keepdims=True), (r1 - r0, 128))

    def qk_unit(u, split):
        if split:
            qk(u, 0, M - LAST)
            qk(u, M - LAST, M)
        else:
            qk(u, 0, M)

    kstep = jnp.minimum(t + 1, NS - 2)

    def prefetch_unit(u):
        v_copy(t, nslot, u).start()
        q_copy(kstep, nslot, u).start()
        k_copy(kstep, nslot, u).start()

    def prefetch():
        for u in range(NG):
            prefetch_unit(u)

    def wait_unit(u):
        v_copy(t - 1, slot, u).wait()
        q_copy(t, slot, u).wait()
        k_copy(t, slot, u).wait()

    @pl.when(t == 0)
    def _():
        for u in range(NG):
            q_copy(0, 0, u).start()
            k_copy(0, 0, u).start()
        for u in range(NG):
            q_copy(0, 0, u).wait()
            k_copy(0, 0, u).wait()
            prefetch_unit(u)
            qk_unit(u, True)

    @pl.when(jnp.logical_and(t > 0, t <= NB))
    def _():
        for u in range(NG):
            wait_unit(u)
            prefetch_unit(u)
            pv(u)
            qk_unit(u, True)

    @pl.when(jnp.logical_and(t > NB, t < NS - 1))
    def _():
        for u in range(NG):
            wait_unit(u)
        prefetch()
        for u in range(NG):
            pv(u)
        for u in range(NG):
            qk_unit(u, u == NG - 1)

    @pl.when(t == NS - 1)
    def _():
        for u in range(NG):
            v_copy(t - 1, slot, u).wait()
            q_copy(t - 1, slot, u).wait()
            k_copy(t - 1, slot, u).wait()
        for u in range(NG):
            pv(u)


@jax.jit
def pallas_standalone__gqa_softmax__near_ridge_kernel(q, k, v):
    B, Hq, Sq, D = q.shape
    Hkv, Sk = k.shape[1], k.shape[2]
    rep = Hq // Hkv
    G = B * Hkv
    M = rep * Sq
    NS = G // NG + 1
    q3 = q.reshape(G, M, D)
    k3 = k.reshape(G, Sk, D)
    v3 = v.reshape(G, Sk, D)
    iv = lambda t: (jnp.maximum(t - 1, 0), 0, 0)
    out = pl.pallas_call(
        functools.partial(_kernel, scale=(D ** -0.5) * math.log2(math.e), NS=NS),
        grid=(NS,),
        in_specs=[
            pl.BlockSpec(memory_space=pl.ANY),
            pl.BlockSpec(memory_space=pl.ANY),
            pl.BlockSpec(memory_space=pl.ANY),
        ],
        out_specs=pl.BlockSpec((NG, M, D), iv),
        out_shape=jax.ShapeDtypeStruct((G, M, D), q.dtype),
        scratch_shapes=[
            pltpu.VMEM((2, NG, M, D), q.dtype),
            pltpu.VMEM((2, NG, Sk, D), k.dtype),
            pltpu.VMEM((2, NG, Sk, D), v.dtype),
            pltpu.VMEM((NG, M, Sk), jnp.float32),
            pltpu.VMEM((NG, M, 128), jnp.float32),
            pltpu.SemaphoreType.DMA((2, NG)),
            pltpu.SemaphoreType.DMA((2, NG)),
            pltpu.SemaphoreType.DMA((2, NG)),
        ],
        compiler_params=pltpu.CompilerParams(
            dimension_semantics=("arbitrary",),
            vmem_limit_bytes=100 * 1024 * 1024,
            disable_bounds_checks=True,
        ),
    )(q3, k3, v3)
    return out.reshape(B, Hq, Sq, D)
```

```python
import functools
import math

import jax
import jax.numpy as jnp
import jax.experimental.pallas as pl
import jax.experimental.pallas.tpu as pltpu

KC = 256
NG = 4
NB = 6
LAST = 128
_NT = (((1,), (1,)), ((), ()))


def _kernel(q_hbm, k_hbm, v_hbm, o_ref, qbuf, kbuf, vbuf, s_ref, m_ref,
            qsem, ksem, vsem, *, scale, NS):
    t = pl.program_id(0)
    _, M, Sk = s_ref.shape
    nk = Sk // KC
    slot = t % 2
    nslot = 1 - slot

    def q_copy(step, sl, u):
        return pltpu.make_async_copy(q_hbm.at[step * NG + u], qbuf.at[sl, u], qsem.at[sl, u])

    def k_copy(step, sl, u):
        return pltpu.make_async_copy(k_hbm.at[step * NG + u], kbuf.at[sl, u], ksem.at[sl, u])

    def v_copy(step, sl, u):
        return pltpu.make_async_copy(v_hbm.at[step * NG + u], vbuf.at[sl, u], vsem.at[sl, u])

    def pv(u):
        m = m_ref[u]
        mt = jnp.concatenate([m] * (KC // 128), axis=1)
        o = None
        l = None
        for j in range(nk):
            p = jnp.exp2(s_ref[u, :, j * KC:(j + 1) * KC] - mt)
            for c in range(KC // 128):
                pc = p[:, c * 128:(c + 1) * 128]
                l = pc if l is None else l + pc
            d = jnp.dot(p.astype(vbuf.dtype), vbuf[slot, u, j * KC:(j + 1) * KC, :],
                        preferred_element_type=jnp.float32)
            o = d if o is None else o + d
        l = jnp.sum(l, axis=-1, keepdims=True)
        o_ref[u] = (o / l).astype(o_ref.dtype)

    def qk(u, r0, r1):
        s = jax.lax.dot_general(qbuf[slot, u, r0:r1, :], kbuf[slot, u], _NT,
                                preferred_element_type=jnp.float32) * scale
        s_ref[u, r0:r1, :] = s
        m_ref[u, r0:r1, :] = jnp.broadcast_to(
            jnp.max(s, axis=-1, keepdims=True), (r1 - r0, 128))

    def qk_unit(u, split):
        if split:
            qk(u, 0, M - LAST)
            qk(u, M - LAST, M)
        else:
            qk(u, 0, M)

    kstep = jnp.minimum(t + 1, NS - 2)

    def prefetch_unit(u):
        v_copy(t, nslot, u).start()
        q_copy(kstep, nslot, u).start()
        k_copy(kstep, nslot, u).start()

    def wait_unit(u):
        v_copy(t - 1, slot, u).wait()
        q_copy(t, slot, u).wait()
        k_copy(t, slot, u).wait()

    @pl.when(t == 0)
    def _():
        for u in range(NG):
            q_copy(0, 0, u).start()
            k_copy(0, 0, u).start()
        for u in range(NG):
            q_copy(0, 0, u).wait()
            k_copy(0, 0, u).wait()
            prefetch_unit(u)
            qk_unit(u, True)

    @pl.when(jnp.logical_and(t > 0, t <= NB))
    def _():
        for u in range(NG):
            wait_unit(u)
            prefetch_unit(u)
            pv(u)
            qk_unit(u, True)

    @pl.when(jnp.logical_and(t > NB, t < NS - 1))
    def _():
        for u in range(NG):
            wait_unit(u)
        for u in range(NG):
            prefetch_unit(u)
        for u in range(NG):
            pv(u)
        for u in range(NG):
            qk_unit(u, u == NG - 1)

    @pl.when(t == NS - 1)
    def _():
        for u in range(NG):
            v_copy(t - 1, slot, u).wait()
            q_copy(t - 1, slot, u).wait()
            k_copy(t - 1, slot, u).wait()
        for u in range(NG):
            pv(u)


@jax.jit
def pallas_standalone__gqa_softmax__near_ridge_kernel(
    q: jax.Array,
    k: jax.Array,
    v: jax.Array,
):
    B, Hq, Sq, D = q.shape
    Hkv, Sk = k.shape[1], k.shape[2]
    rep = Hq // Hkv
    G = B * Hkv
    M = rep * Sq
    assert G % NG == 0 and Sk % KC == 0 and M > LAST and (M - LAST) % 16 == 0
    NS = G // NG + 1
    assert NB < NS - 1
    q3 = q.reshape(G, M, D)
    k3 = k.reshape(G, Sk, D)
    v3 = v.reshape(G, Sk, D)
    out = pl.pallas_call(
        functools.partial(_kernel, scale=(D ** -0.5) * math.log2(math.e), NS=NS),
        grid=(NS,),
        in_specs=[
            pl.BlockSpec(memory_space=pl.ANY),
            pl.BlockSpec(memory_space=pl.ANY),
            pl.BlockSpec(memory_space=pl.ANY),
        ],
        out_specs=pl.BlockSpec((NG, M, D), lambda t: (jnp.maximum(t - 1, 0), 0, 0)),
        out_shape=jax.ShapeDtypeStruct((G, M, D), q.dtype),
        scratch_shapes=[
            pltpu.VMEM((2, NG, M, D), q.dtype),
            pltpu.VMEM((2, NG, Sk, D), k.dtype),
            pltpu.VMEM((2, NG, Sk, D), v.dtype),
            pltpu.VMEM((NG, M, Sk), jnp.float32),
            pltpu.VMEM((NG, M, 128), jnp.float32),
            pltpu.SemaphoreType.DMA((2, NG)),
            pltpu.SemaphoreType.DMA((2, NG)),
            pltpu.SemaphoreType.DMA((2, NG)),
        ],
        compiler_params=pltpu.CompilerParams(
            dimension_semantics=("arbitrary",),
            vmem_limit_bytes=100 * 1024 * 1024,
            disable_bounds_checks=True,
        ),
    )(q3, k3, v3)
    return out.reshape(B, Hq, Sq, D)
```

```python
import functools
import math

import jax
import jax.numpy as jnp
import jax.experimental.pallas as pl
import jax.experimental.pallas.tpu as pltpu

KC = 256
NG = 4
NB = 2
NB2 = 8
LAST = 128
_NT = (((1,), (1,)), ((), ()))


def _kernel(q_hbm, k_hbm, v_hbm, o_ref, qbuf, kbuf, vbuf, s_ref, m_ref,
            qsem, ksem, vsem, *, scale, NS):
    t = pl.program_id(0)
    _, M, Sk = s_ref.shape
    nk = Sk // KC
    slot = t % 2
    nslot = 1 - slot

    def q_copy(step, sl, u):
        return pltpu.make_async_copy(q_hbm.at[step * NG + u], qbuf.at[sl, u], qsem.at[sl, u])

    def k_copy(step, sl, u):
        return pltpu.make_async_copy(k_hbm.at[step * NG + u], kbuf.at[sl, u], ksem.at[sl, u])

    def v_copy(step, sl, u):
        return pltpu.make_async_copy(v_hbm.at[step * NG + u], vbuf.at[sl, u], vsem.at[sl, u])

    def pv(u):
        m = m_ref[u]
        mt = jnp.concatenate([m] * (KC // 128), axis=1)
        o = None
        l = None
        for j in range(nk):
            p = jnp.exp2(s_ref[u, :, j * KC:(j + 1) * KC] - mt)
            for c in range(KC // 128):
                pc = p[:, c * 128:(c + 1) * 128]
                l = pc if l is None else l + pc
            d = jnp.dot(p.astype(vbuf.dtype), vbuf[slot, u, j * KC:(j + 1) * KC, :],
                        preferred_element_type=jnp.float32)
            o = d if o is None else o + d
        l = jnp.sum(l, axis=-1, keepdims=True)
        o_ref[u] = (o / l).astype(o_ref.dtype)

    def lane_max(m):
        return jnp.broadcast_to(jnp.max(m, axis=-1, keepdims=True), m.shape)

    def qk(u, r0, r1, final=True):
        s = jax.lax.dot_general(qbuf[slot, u, r0:r1, :], kbuf[slot, u], _NT,
                                preferred_element_type=jnp.float32) * scale
        s_ref[u, r0:r1, :] = s
        m = s[:, 0:128]
        for c in range(1, Sk // 128):
            m = jnp.maximum(m, s[:, c * 128:(c + 1) * 128])
        m_ref[u, r0:r1, :] = lane_max(m) if final else m

    def qk_unit(u, mode):
        if mode == "split":
            qk(u, 0, M - LAST)
            qk(u, M - LAST, M)
        elif mode == "defer":
            qk(u, 0, M, final=False)
        else:
            qk(u, 0, M)

    def finalize(u):
        m_ref[u] = lane_max(m_ref[u])

    kstep = jnp.minimum(t + 1, NS - 2)

    def prefetch_unit(u):
        v_copy(t, nslot, u).start()
        q_copy(kstep, nslot, u).start()
        k_copy(kstep, nslot, u).start()

    def wait_unit(u):
        v_copy(t - 1, slot, u).wait()
        q_copy(t, slot, u).wait()
        k_copy(t, slot, u).wait()

    def region(us, fin, last_mode):
        for u in us:
            wait_unit(u)
        for u in us:
            prefetch_unit(u)
        for u in us:
            pv(u)
        if fin is not None:
            finalize(fin)
        for i, u in enumerate(us):
            qk_unit(u, last_mode if i == len(us) - 1 else "full")

    @pl.when(t == 0)
    def _():
        for u in range(NG):
            q_copy(0, 0, u).start()
            k_copy(0, 0, u).start()
        q_copy(0, 0, 0).wait()
        k_copy(0, 0, 0).wait()
        prefetch_unit(0)
        qk_unit(0, "defer")

        def first(u, carry):
            q_copy(0, 0, u).wait()
            k_copy(0, 0, u).wait()
            prefetch_unit(u)
            finalize(u - 1)
            qk_unit(u, "defer")
            return carry
        jax.lax.fori_loop(1, NG, first, 0)

    @pl.when(jnp.logical_and(t > 0, t <= NB))
    def _():
        def one(u, carry):
            region([u], (u + NG - 1) % NG, "defer")
            return carry
        jax.lax.fori_loop(0, NG, one, 0)

    @pl.when(jnp.logical_and(t > NB, t <= NB2))
    def _():
        def two(g, carry):
            region([2 * g, 2 * g + 1], (2 * g + NG - 1) % NG, "defer")
            return carry
        jax.lax.fori_loop(0, NG // 2, two, 0)

    @pl.when(t == NB2 + 1)
    def _():
        finalize(NG - 1)

    @pl.when(jnp.logical_and(t > NB2, t < NS - 1))
    def _():
        region(list(range(NG)), None, "split")

    @pl.when(t == NS - 1)
    def _():
        for u in range(NG):
            v_copy(t - 1, slot, u).wait()
            q_copy(t - 1, slot, u).wait()
            k_copy(t - 1, slot, u).wait()
        for u in range(NG):
            pv(u)


@jax.jit
def pallas_standalone__gqa_softmax__near_ridge_kernel(
    q: jax.Array,
    k: jax.Array,
    v: jax.Array,
):
    B, Hq, Sq, D = q.shape
    Hkv, Sk = k.shape[1], k.shape[2]
    rep = Hq // Hkv
    G = B * Hkv
    M = rep * Sq
    assert G % NG == 0 and Sk % KC == 0 and M > LAST and (M - LAST) % 16 == 0
    NS = G // NG + 1
    assert NG == 4 and 1 <= NB < NB2 < NS - 1
    q3 = q.reshape(G, M, D)
    k3 = k.reshape(G, Sk, D)
    v3 = v.reshape(G, Sk, D)
    out = pl.pallas_call(
        functools.partial(_kernel, scale=(D ** -0.5) * math.log2(math.e), NS=NS),
        grid=(NS,),
        in_specs=[
            pl.BlockSpec(memory_space=pl.ANY),
            pl.BlockSpec(memory_space=pl.ANY),
            pl.BlockSpec(memory_space=pl.ANY),
        ],
        out_specs=pl.BlockSpec((NG, M, D), lambda t: (jnp.maximum(t - 1, 0), 0, 0)),
        out_shape=jax.ShapeDtypeStruct((G, M, D), q.dtype),
        scratch_shapes=[
            pltpu.VMEM((2, NG, M, D), q.dtype),
            pltpu.VMEM((2, NG, Sk, D), k.dtype),
            pltpu.VMEM((2, NG, Sk, D), v.dtype),
            pltpu.VMEM((NG, M, Sk), jnp.float32),
            pltpu.VMEM((NG, M, 128), jnp.float32),
            pltpu.SemaphoreType.DMA((2, NG)),
            pltpu.SemaphoreType.DMA((2, NG)),
            pltpu.SemaphoreType.DMA((2, NG)),
        ],
        compiler_params=pltpu.CompilerParams(
            dimension_semantics=("arbitrary",),
            vmem_limit_bytes=100 * 1024 * 1024,
            disable_bounds_checks=True,
        ),
    )(q3, k3, v3)
    return out.reshape(B, Hq, Sq, D)
```
